```python
import os as _os
_os.environ.setdefault('JAX_PLATFORMS', 'cpu')
import jax
import jax.numpy as jnp

def _softmax(x, axis=-1):
    return jax.nn.softmax(x, axis=axis)

def _gelu(x):
    return jax.nn.gelu(x, approximate=True)

def _silu(x):
    return jax.nn.silu(x)

def _sigmoid(x):
    return jax.nn.sigmoid(x)

def _layernorm(x, axis=-1, eps=1e-05):
    m = jnp.mean(x, axis=axis, keepdims=True)
    v = jnp.var(x, axis=axis, keepdims=True)
    return (x - m) / jnp.sqrt(v + eps)

def _scatter_add(tgt, idx, src, axis=0):
    return tgt.at[idx].add(src)

def _segment_sum(src, seg, n):
    return jax.ops.segment_sum(src, seg, n)

class _Rng:

    def __init__(self, key):
        self._k = key

    def _next(self):
        self._k, sub = jax.random.split(self._k)
        return sub

    def normal(self, shape):
        return jax.random.normal(self._next(), shape, dtype=jnp.bfloat16)

    def randint(self, lo, hi, shape):
        return jax.random.randint(self._next(), shape, lo, hi, dtype=jnp.int32)

    def uniform(self, shape, lo=0.0, hi=1.0):
        return jax.random.uniform(self._next(), shape, jnp.bfloat16, lo, hi)

    def permutation(self, n):
        return jax.random.permutation(self._next(), n)
kernel_name = 'gated_mix__mha_block__memory_aug_recurrent_mem_tr__prompt'

def setup_inputs():
    _rng = _Rng(jax.random.key(int.from_bytes(__import__("os").urandom(4), "little")))
    _w = lambda a: (lambda t: t.astype(jnp.bfloat16) if jnp.issubdtype(t.dtype, jnp.floating) else t)(jnp.asarray(a))

    def _A_setup():
        B, S, D, H = (1, 2048, 512, 32)
        return {'x': _w((lambda *s: _rng.normal(s) * 0.05)(B, S, D)), 'wqkv': _w((lambda *s: _rng.normal(s) * 0.8)(D, 3 * D)), 'wo': _w((lambda *s: _rng.normal(s) * 0.05)(D, D))}
    _A_in = _A_setup()

    def _B_setup():
        B, S, Dm = (1, 2048, 512)
        H, Dh = (32, 128)
        M, seg = (8, 32)
        seg = min(seg, S)
        S = S // seg * seg
        return {'x': _w((lambda *s: _rng.normal(s) * 0.05)(B, S, Dm)), 'mem0': _w((lambda *s: _rng.normal(s) * 0.8)(B, M, Dm)), 'Wq': _w((lambda *s: _rng.normal(s) * 1.6)(Dm, H, Dh) * Dm ** (-0.5)), 'Wk': _w((lambda *s: _rng.normal(s) * 1.6)(Dm, H, Dh) * Dm ** (-0.5)), 'Wv': _w((lambda *s: _rng.normal(s) * 0.8)(Dm, H, Dh) * Dm ** (-0.5)), 'Wo': _w((lambda *s: _rng.normal(s) * 0.8)(H, Dh, Dm) * (H * Dh) ** (-0.5)), 'seg_len': seg}
    _B_in = _B_setup()
    return {'A_x': _A_in['x'], 'A_wqkv': _A_in['wqkv'], 'A_wo': _A_in['wo'], 'B_x': _B_in['x'], 'B_mem0': _B_in['mem0'], 'B_Wq': _B_in['Wq'], 'B_Wk': _B_in['Wk'], 'B_Wv': _B_in['Wv'], 'B_Wo': _B_in['Wo'], 'B_seg_len': _B_in['seg_len'], 'gate_w': _w((lambda *s: _rng.normal(s) * 0.05)(512) * 16.0)}

def reference(A_x, A_wqkv, A_wo, B_x, B_mem0, B_Wq, B_Wk, B_Wv, B_Wo, B_seg_len, gate_w):

    def _A_ref(x, wqkv, wo):
        B, S, D = x.shape
        H = 32
        Dh = D // H
        qkv = (lambda x, *d: x.transpose(*d))((x @ wqkv).reshape(B, S, 3, H, Dh), 2, 0, 3, 1, 4)
        q, k, v = (qkv[0], qkv[1], qkv[2])
        scores = jnp.einsum('bhqd,bhkd->bhqk', q, k) * Dh ** (-0.5)
        p = _softmax(scores, axis=-1)
        o = jnp.einsum('bhqk,bhkd->bhqd', p, v)
        return (lambda x, *d: x.transpose(*d))(o, 0, 2, 1, 3).reshape(B, S, D) @ wo

    def _B_ref(x, mem0, Wq, Wk, Wv, Wo, seg_len):
        B, S, Dm = x.shape
        H, Dh = (Wq.shape[1], Wq.shape[2])
        M = mem0.shape[1]
        scale = Dh ** (-0.5)
        n_seg = S // seg_len
        L = M + seg_len
        idx = jnp.arange(L)
        mask = (idx[:, None] < M) | (idx[:, None] >= idx[None, :])
        mem = mem0
        outs = []
        for s in range(n_seg):
            xs = x[:, s * seg_len:(s + 1) * seg_len, :].copy()
            h = jnp.concatenate([mem, xs], axis=1)
            q = jnp.einsum('btd,dhe->bhte', h, Wq)
            k = jnp.einsum('btd,dhe->bhte', h, Wk)
            v = jnp.einsum('btd,dhe->bhte', h, Wv)
            scores = jnp.einsum('bhqe,bhke->bhqk', q, k) * scale
            scores = jnp.where(mask[None, None], scores, -1000000000.0)
            p = _softmax(scores, axis=-1)
            o = jnp.einsum('bhqk,bhke->bhqe', p, v)
            o = jnp.einsum('bhte,hed->btd', o, Wo)
            mem = o[:, :M, :].copy()
            outs.append(o[:, M:, :])
        return jnp.concatenate(outs, axis=1)
    x = A_x
    g = _sigmoid((x * gate_w).sum(-1, keepdims=True))
    a = _A_ref(x, A_wqkv, A_wo)
    b = _B_ref(x, B_mem0, B_Wq, B_Wk, B_Wv, B_Wo, B_seg_len)
    return g * a + (1 - g) * b
```

```python
import functools
import math

import jax
import jax.numpy as jnp
import numpy as np
from jax import lax
from jax.experimental import pallas as pl
from jax.experimental.pallas import tpu as pltpu

BF = jnp.bfloat16
F32 = jnp.float32
U32 = jnp.uint32
LOG2E = math.log2(math.e)

S_, D_ = 2048, 512
HA, DA = 32, 16
HB, DB = 32, 128
MEM, SEG = 8, 32
NSEG = S_ // SEG
QB = 512
NQB = S_ // QB
KC = 128
G = 4
NCH = 16


def _nn(a, b):
    return lax.dot_general(a, b, (((1,), (0,)), ((), ())), preferred_element_type=F32)


def _nt(a, b):
    return lax.dot_general(a, b, (((1,), (1,)), ((), ())), preferred_element_type=F32)


def _tn(a, b):
    return lax.dot_general(a, b, (((0,), (0,)), ((), ())), preferred_element_type=F32)


def _kernel(x_ref, wqkv_ref, wo_ref, mem0_ref, gw_ref,
            wq_hbm, wk_hbm, wv_hbm, wo2_hbm,
            o_ref,
            st_q, st_k, st_v, st_o, w3, wo2, qt_ref, kc_ref, vt_ref, ot_ref,
            ga_ref, omg_ref, s_a, s_b, sems):
    copies = [
        pltpu.make_async_copy(wq_hbm, st_q, sems.at[0]),
        pltpu.make_async_copy(wk_hbm, st_k, sems.at[1]),
        pltpu.make_async_copy(wv_hbm, st_v, sems.at[2]),
        pltpu.make_async_copy(wo2_hbm, st_o, sems.at[3]),
    ]
    for c in copies:
        c.start()

    qscale = (DA ** -0.5) * LOG2E
    wq = wqkv_ref[:, 0:D_]
    wk = wqkv_ref[:, D_:2 * D_]
    wv = wqkv_ref[:, 2 * D_:3 * D_]
    for qb in range(NQB):
      with jax.named_scope("A0"):
        xb = x_ref[qb * QB:(qb + 1) * QB, :]
        kk = _nn(xb, wk).astype(BF)
        for g in range(4):
            kc_ref[g, qb * QB:(qb + 1) * QB, :] = kk[:, g * 128:(g + 1) * 128]
        qT = lax.dot_general(wq, xb, (((0,), (1,)), ((), ())),
                             preferred_element_type=F32)
        qt_ref[qb] = (qT * qscale).astype(BF)
        vT = lax.dot_general(wv, xb, (((0,), (1,)), ((), ())),
                             preferred_element_type=F32)
        vt_ref[:, qb * QB:(qb + 1) * QB] = vT.astype(BF)
        xf = xb.astype(F32)
        gl = jnp.sum(xf * gw_ref[...].astype(F32), axis=1, keepdims=True)
        gate = 1.0 / (1.0 + jnp.exp(-gl))
        omg_ref[qb * QB:(qb + 1) * QB, :] = jnp.broadcast_to(gate, (QB, 128))

    r16 = lax.broadcasted_iota(jnp.int32, (16, S_), 0)
    ones_aug = jnp.where(r16 == 0, 1.0, 0.0).astype(BF)
    rowhead = lax.broadcasted_iota(jnp.int32, (128, QB), 0) // DA

    NKC = S_ // KC

    def a_q(u):
        h = u // NQB
        qb = u % NQB
        g = h // 8
        j = h % 8
        qt = qt_ref[qb, pl.ds(pl.multiple_of(g * 128, 128), 128), :]
        return g, jnp.where(rowhead == j, qt, jnp.zeros_like(qt))

    def a_s1(g, qm, sbuf, kc, mrun):
        kg = kc_ref[g, kc * KC:(kc + 1) * KC, :]
        sT = _nn(kg, qm)
        sbuf[kc * KC:(kc + 1) * KC, :] = sT
        mp = jnp.max(sT.reshape(KC // 8, 8, QB), axis=0)
        return mp if mrun is None else jnp.maximum(mrun, mp)

    def a_s2(h, sbuf, kc, m, acc):
        sT = sbuf[kc * KC:(kc + 1) * KC, :]
        pT = jnp.exp2(sT - m).astype(BF)
        vt = vt_ref[pl.ds(pl.multiple_of(h * DA, DA), DA), kc * KC:(kc + 1) * KC]
        vta = jnp.concatenate([vt, ones_aug[:, 0:KC]], axis=0)
        d = _nn(vta, pT)
        return d if acc is None else acc + d

    def a_fin(u, acc):
        h = u // NQB
        qb = u % NQB
        l = acc[16:17, :]
        r = pl.reciprocal(l, approx=True)
        r = r * (2.0 - l * r)
        o = acc[0:16, :] * r
        ot_ref[qb, pl.ds(pl.multiple_of(h * DA, DA), DA), :] = o.astype(BF)

    def a_pair(u1, sb1, u2, sb2, m):
        if u1 is not None:
            g, qm = a_q(u1)
        mrun = None
        acc = None
        for kc in range(NKC):
            if u1 is not None:
                mrun = a_s1(g, qm, sb1, kc, mrun)
            if u2 is not None:
                acc = a_s2(u2 // NQB, sb2, kc, m, acc)
        if u2 is not None:
            a_fin(u2, acc)
        if u1 is not None:
            return jnp.max(mrun, axis=0, keepdims=True)
        return None

    NU = HA * NQB
    with jax.named_scope("A1"):
        m0 = a_pair(0, s_a, None, None, None)

        def a_body(i, m):
            m = a_pair(2 * i + 1, s_b, 2 * i, s_a, m)
            m = a_pair(2 * i + 2, s_a, 2 * i + 1, s_b, m)
            return m

        m = lax.fori_loop(0, NU // 2 - 1, a_body, m0)
        m = a_pair(NU - 1, s_b, NU - 2, s_a, m)
        a_pair(None, None, NU - 1, s_b, m)

    for qb in range(NQB):
      with jax.named_scope("A2"):
        a = _tn(ot_ref[qb], wo_ref[...])
        gate = omg_ref[qb * QB:(qb + 1) * QB, :]
        gt = jnp.concatenate([gate] * 4, axis=1)
        ga_ref[qb * QB:(qb + 1) * QB, :] = a * gt
        omg_ref[qb * QB:(qb + 1) * QB, :] = 1.0 - gate

    for c in copies:
        c.wait()
    CH = 256 // NCH

    def relayout(ci, carry):
        ob = pl.multiple_of(ci * CH, CH)
        for t, st in enumerate((st_q, st_k, st_v)):
            w32 = st.at[ci].bitcast(U32)
            for j in range(16):
                a = w32[pl.ds(j, CH, stride=32), :]
                b = w32[pl.ds(16 + j, CH, stride=32), :]
                ev = (a & U32(0xFFFF)) | (b << 16)
                od = (a >> 16) | (b & U32(0xFFFF0000))
                w3[2 * j, pl.ds(ob, CH), t * 128:(t + 1) * 128] = ev
                w3[2 * j + 1, pl.ds(ob, CH), t * 128:(t + 1) * 128] = od
        return carry

    with jax.named_scope("relayout"):
        lax.fori_loop(0, NCH, relayout, 0)

    def relayout_o(h, carry):
        wo2[h] = pltpu.bitcast(st_o[h], U32)
        return carry

    lax.fori_loop(0, HB, relayout_o, 0)

    bscale = (DB ** -0.5) * LOG2E
    ri = lax.broadcasted_iota(jnp.int32, (48, 128), 0)
    ci_ = lax.broadcasted_iota(jnp.int32, (48, 128), 1)
    allowed = (ri >= SEG) | (ci_ >= SEG) | (ci_ <= ri)
    padcol = ci_ >= SEG + MEM
    zeros8 = jnp.zeros((8, D_), F32)

    fill = jnp.where(padcol, -jnp.inf, -1e9 * LOG2E).astype(F32)
    keep = jnp.logical_and(allowed, jnp.logical_not(padcol))

    def b_step(s, mem):
        r0 = pl.multiple_of(s * SEG, SEG)
        xs = x_ref[pl.ds(r0, SEG), :]
        mp = jnp.concatenate([mem, zeros8], axis=0).astype(BF)
        h = jnp.concatenate([xs, mp], axis=0)
        NG = HB // G
        st1, st2, st3, st4 = {}, {}, {}, {}
        acc = jnp.zeros((48, D_), F32)

        def s1(g):
            out = []
            for hd in range(g * G, (g + 1) * G):
                w = pltpu.bitcast(w3[hd], BF)
                qkv = _nn(h, w)
                q = (qkv[:, 0:128] * bscale).astype(BF)
                k = qkv[:, 128:256].astype(BF)
                v = qkv[:, 256:384].astype(BF)
                out.append((q, k, v))
            st1[g] = out

        def s2(g):
            out = []
            for (q, k, v) in st1.pop(g):
                sc = _nt(q, k)
                sc = jnp.where(keep[:, 0:48], sc, fill[:, 0:48])
                mx = jnp.max(sc, axis=1, keepdims=True)
                out.append((sc, mx, v))
            st2[g] = out

        def s3(g):
            out = []
            for (sc, mx, v) in st2.pop(g):
                e = jnp.exp2(sc - mx)
                l = jnp.sum(e, axis=1, keepdims=True)
                out.append((e.astype(BF), l, v))
            st3[g] = out

        def s4(g):
            out = []
            for (e, l, v) in st3.pop(g):
                o = _nn(e, v)
                r = pl.reciprocal(l, approx=True)
                r = r * (2.0 - l * r)
                out.append((o, r))
            st4[g] = out

        def s5(g, acc):
            for hl, (o, r) in enumerate(st4.pop(g)):
                hd = g * G + hl
                wo_h = pltpu.bitcast(wo2[hd], BF)
                acc = acc + _nn((o * r).astype(BF), wo_h)
            return acc

        for t in range(NG + 4):
            if t < NG:
                s1(t)
            if 0 <= t - 1 < NG:
                s2(t - 1)
            if 0 <= t - 2 < NG:
                s3(t - 2)
            if 0 <= t - 3 < NG:
                s4(t - 3)
            if 0 <= t - 4 < NG:
                acc = s5(t - 4, acc)
        b = acc[0:SEG, :]
        om = omg_ref[pl.ds(r0, SEG), :]
        omt = jnp.concatenate([om] * 4, axis=1)
        o_ref[pl.ds(r0, SEG), :] = (ga_ref[pl.ds(r0, SEG), :] + omt * b).astype(o_ref.dtype)
        return acc[SEG:SEG + MEM, :].astype(BF).astype(F32)

    with jax.named_scope("B"):
        lax.fori_loop(0, NSEG, b_step, mem0_ref[...].astype(F32))


def pallas_gated_mix__mha_block__memory_aug_recurrent_mem_tr__prompt_kernel(
        A_x, A_wqkv, A_wo, B_x, B_mem0, B_Wq, B_Wk, B_Wv, B_Wo, B_seg_len, gate_w):
    del B_x
    assert B_seg_len == SEG
    x = A_x.reshape(S_, D_)
    mem0 = B_mem0.reshape(MEM, D_)
    gw = gate_w.reshape(1, D_)
    wq = B_Wq.reshape(NCH, D_ * HB // NCH, DB)
    wk = B_Wk.reshape(NCH, D_ * HB // NCH, DB)
    wv = B_Wv.reshape(NCH, D_ * HB // NCH, DB)
    vm = pl.BlockSpec(memory_space=pltpu.VMEM)
    hbm = pl.BlockSpec(memory_space=pl.ANY)
    out = pl.pallas_call(
        _kernel,
        out_shape=jax.ShapeDtypeStruct((S_, D_), A_x.dtype),
        in_specs=[vm, vm, vm, vm, vm, hbm, hbm, hbm, hbm],
        out_specs=vm,
        scratch_shapes=[
            pltpu.VMEM((NCH, D_ * HB // NCH, DB), BF),
            pltpu.VMEM((NCH, D_ * HB // NCH, DB), BF),
            pltpu.VMEM((NCH, D_ * HB // NCH, DB), BF),
            pltpu.VMEM((HB, DB, D_), BF),
            pltpu.VMEM((HB, D_ // 2, 3 * DB), U32),
            pltpu.VMEM((HB, DB // 2, D_), U32),
            pltpu.VMEM((NQB, D_, QB), BF),
            pltpu.VMEM((4, S_, 128), BF),
            pltpu.VMEM((D_, S_), BF),
            pltpu.VMEM((NQB, D_, QB), BF),
            pltpu.VMEM((S_, D_), F32),
            pltpu.VMEM((S_, 128), F32),
            pltpu.VMEM((S_, QB), F32),
            pltpu.VMEM((S_, QB), F32),
            pltpu.SemaphoreType.DMA((4,)),
        ],
        compiler_params=pltpu.CompilerParams(vmem_limit_bytes=100 * 1024 * 1024),
    )(x, A_wqkv, A_wo, mem0, gw, wq, wk, wv, B_Wo)
    return out.reshape(1, S_, D_)
```

```python
import functools
import math

import jax
import jax.numpy as jnp
import numpy as np
from jax import lax
from jax.experimental import pallas as pl
from jax.experimental.pallas import tpu as pltpu

BF = jnp.bfloat16
F32 = jnp.float32
U32 = jnp.uint32
LOG2E = math.log2(math.e)

S_, D_ = 2048, 512
HA, DA = 32, 16
HB, DB = 32, 128
MEM, SEG = 8, 32
NSEG = S_ // SEG
QB = 512
NQB = S_ // QB
LAG = 2
RELMERGE = 1
SUMMODE = 1
F32ATT = 1
UL = 2
KC = 128
G = 4
NCH = 32


def _nn(a, b):
    return lax.dot_general(a, b, (((1,), (0,)), ((), ())), preferred_element_type=F32)


def _nt(a, b):
    return lax.dot_general(a, b, (((1,), (1,)), ((), ())), preferred_element_type=F32)


def _tn(a, b):
    return lax.dot_general(a, b, (((0,), (0,)), ((), ())), preferred_element_type=F32)


def _kernel(x_ref, wqkv_ref, wo_ref, mem0_ref, gw_ref,
            wq_hbm, wk_hbm, wv_hbm, wo2_hbm,
            o_ref,
            st_q, st_k, st_v, st_o, w3, wo2, qt_ref, kc_ref, vt_ref, ot_ref,
            ga_ref, omg_ref, s_a, s_b, kr_ref, xl_ref, ql_ref, ol_ref, bl_ref, m_ref, sems):
    copies = [
        pltpu.make_async_copy(wq_hbm, st_q, sems.at[0]),
        pltpu.make_async_copy(wk_hbm, st_k, sems.at[1]),
        pltpu.make_async_copy(wv_hbm, st_v, sems.at[2]),
        pltpu.make_async_copy(wo2_hbm, st_o, sems.at[3]),
    ]
    for c in copies:
        c.start()

    qscale = (DA ** -0.5) * LOG2E
    wq = wqkv_ref[:, 0:D_]
    wk = wqkv_ref[:, D_:2 * D_]
    wv = wqkv_ref[:, 2 * D_:3 * D_]
    def a0_block(qb, carry):
        r0 = pl.multiple_of(qb * QB, QB)
        xb = x_ref[pl.ds(r0, QB), :]
        kk = _nn(xb, wk).astype(BF)
        for g in range(4):
            kc_ref[g, pl.ds(pl.multiple_of(qb * (QB // 2), QB // 2), QB // 2), :] = pltpu.bitcast(kk[:, g * 128:(g + 1) * 128], U32)
        qT = lax.dot_general(wq, xb, (((0,), (1,)), ((), ())),
                             preferred_element_type=F32)
        qt_ref[qb] = (qT * qscale).astype(BF)
        vT = lax.dot_general(wv, xb, (((0,), (1,)), ((), ())),
                             preferred_element_type=F32)
        vt_ref[qb] = vT.astype(BF)
        xf = xb.astype(F32)
        gl = jnp.sum(xf * gw_ref[...].astype(F32), axis=1, keepdims=True)
        gate = 1.0 / (1.0 + jnp.exp(-gl))
        omg_ref[pl.ds(r0, QB), :] = jnp.broadcast_to(gate, (QB, 128))
        return carry

    with jax.named_scope("A0"):
        lax.fori_loop(0, NQB, a0_block, 0)


    NKC = S_ // KC
    NU = HA * NQB
    sbufs = (s_a, s_b)

    def krol_store(hn, c):
        g = hn // 8
        j = hn % 8
        rows = slice(c * (KC // 2), (c + 1) * (KC // 2))
        kr_ref[rows, :] = pltpu.roll(kc_ref[g, rows, :], (128 - DA * j) % 128, 1)

    def a_s1(qh, sbuf, kc, mrun):
        kr = pltpu.bitcast(kr_ref[kc * (KC // 2):(kc + 1) * (KC // 2), :], BF)
        sT = _nn(kr[:, 0:DA], qh)
        sbuf[kc * KC:(kc + 1) * KC, :] = sT
        mp = jnp.max(sT.reshape(KC // 8, 8, QB), axis=0)
        return mp if mrun is None else jnp.maximum(mrun, mp)

    def a_s2(h, sbuf, kc, m, acc, lneg):
        sT = sbuf[kc * KC:(kc + 1) * KC, :]
        e = jnp.exp2(sT - m)
        parts = []
        for r in range(KC // 32 - 1, -1, -1):
            e0, e1, e2, e3 = [e[r * 32 + 8 * i:r * 32 + 8 * i + 8, :] for i in range(4)]
            t = (e0 + e1) + (e2 + e3)
            lneg = -t if lneg is None else lneg - t
            parts.append(jnp.concatenate([jnp.maximum(e0, lneg), e1, e2, e3], axis=0))
        p = jnp.concatenate(parts[::-1], axis=0).astype(BF)
        vt = vt_ref[kc // (QB // KC), pl.ds(pl.multiple_of(h * DA, DA), DA), (kc % (QB // KC)) * KC:(kc % (QB // KC) + 1) * KC]
        d = _nn(vt, p)
        return (d if acc is None else acc + d), lneg

    def a_fin(h, qb, acc, lneg):
        l = -jnp.sum(lneg, axis=0, keepdims=True)
        r = pltpu.reciprocal(l, approx=True)
        r = r * (2.0 - l * r)
        o = acc * r
        ot_ref[qb, pl.ds(pl.multiple_of(h * DA, DA), DA), :] = o.astype(BF)

    def a_units(h, hpy, state, extra=None):
        acc, lneg, m1, m2 = state
        for qb in range(NQB):
            pi = hpy * NQB + qb
            do1 = pi < NU
            if do1:
                qh = qt_ref[qb, pl.ds(pl.multiple_of(h * DA, DA), DA), :]
            mrun = None
            for c in range(NKC):
                if do1:
                    mrun = a_s1(qh, sbufs[pi % 2], c, mrun)
                    if qb == NQB - 1 and hpy < HA - 1:
                        krol_store(h + 1, c)
                if c < LAG:
                    back, c2, mm = 2, NKC - LAG + c, m2
                else:
                    back, c2, mm = 1, c - LAG, m1
                p2 = pi - back
                if 0 <= p2 < NU:
                    qb2 = qb - back
                    h2 = h if qb2 >= 0 else h - 1
                    qb2 = qb2 % NQB
                    if c2 == 0:
                        acc, lneg = None, None
                    acc, lneg = a_s2(h2, sbufs[p2 % 2], c2, mm, acc, lneg)
                    if c2 == NKC - 1:
                        a_fin(h2, qb2, acc, lneg)
                if extra is not None:
                    extra(qb * NKC + c)
            m2 = m1
            m1 = jnp.max(mrun, axis=0, keepdims=True) if do1 else None
            if not do1 and pi >= NU + 1:
                break
        return acc, lneg, m1, m2

    CH = 256 // NCH

    def relayout_piece(ci, slot):
        if slot < 48:
            t, j = slot // 16, slot % 16
            st = (st_q, st_k, st_v)[t]
            w32 = st.at[ci].bitcast(U32)
            ob = pl.multiple_of(ci * CH, CH)
            a = w32[pl.ds(j, CH, stride=32), :]
            b = w32[pl.ds(16 + j, CH, stride=32), :]
            w3[2 * j, pl.ds(ob, CH), t * 128:(t + 1) * 128] = (a & U32(0xFFFF)) | (b << 16)
            w3[2 * j + 1, pl.ds(ob, CH), t * 128:(t + 1) * 128] = (a >> 16) | (b & U32(0xFFFF0000))
        elif slot < 52:
            q = slot - 48
            wo2[ci, q * 16:(q + 1) * 16, :] = pltpu.bitcast(st_o[ci, q * 32:(q + 1) * 32, :], U32)

    with jax.named_scope("A1"):
        for c in range(NKC):
            krol_store(0, c)
        st = a_units(0, 0, (None, None, None, None))
        for cp in copies:
            cp.wait()

        def a_body(i, st):
            if RELMERGE:
                return a_units(i, 1, st, extra=lambda slot: relayout_piece(i - 1, slot))
            return a_units(i, 1, st)

        st = lax.fori_loop(1, HA, a_body, st)
        a_units(HA, HA, st)

    for qb in range(NQB):
      with jax.named_scope("A2"):
        a = _tn(ot_ref[qb], wo_ref[...])
        gate = omg_ref[qb * QB:(qb + 1) * QB, :]
        gt = jnp.concatenate([gate] * 4, axis=1)
        ga_ref[qb * QB:(qb + 1) * QB, :] = a * gt
        omg_ref[qb * QB:(qb + 1) * QB, :] = 1.0 - gate

    with jax.named_scope("relayout"):
        if RELMERGE:
            for slot in range(52):
                relayout_piece(NCH - 1, slot)
        else:
            def relayout(ci, carry):
                for slot in range(52):
                    relayout_piece(ci, slot)
                return carry
            lax.fori_loop(0, NCH, relayout, 0)

    bscale = (DB ** -0.5) * LOG2E
    NE = SEG - MEM
    NL = NSEG * MEM

    with jax.named_scope("BL1"):
        for s in range(NSEG):
            xl_ref[s * MEM:(s + 1) * MEM, :] = x_ref[s * SEG + NE:(s + 1) * SEG, :]

        def bl1(i, carry):
            for hl in range(UL):
                hd = i * UL + hl
                w = pltpu.bitcast(w3[hd], BF)
                qkv = _nn(xl_ref[...], w)
                ql_ref[hd, :, 0:128] = (qkv[:, 0:128] * bscale).astype(BF)
                ql_ref[hd, :, 128:384] = qkv[:, 128:384].astype(BF)
            return carry

        lax.fori_loop(0, HB // UL, bl1, 0)

    if F32ATT:
        LP = 40
    else:
        LP = 48
    ri = lax.broadcasted_iota(jnp.int32, (LP, LP), 0)
    ci_ = lax.broadcasted_iota(jnp.int32, (LP, LP), 1)
    allowed = (ri >= SEG) | (ci_ >= SEG) | (ci_ <= ri)
    padcol = ci_ >= SEG + MEM
    fill = jnp.where(padcol, -jnp.inf, -1e9 * LOG2E).astype(F32)
    keep = jnp.logical_and(allowed, jnp.logical_not(padcol))
    z8 = jnp.zeros((8, 128), F32)

    def b_step(s, mem):
        r0 = pl.multiple_of(s * SEG, SEG)
        l0 = pl.multiple_of(s * MEM, MEM)
        xs = x_ref[pl.ds(r0, SEG), :]
        tail = jnp.concatenate([xs[16:SEG, :].astype(F32)[0:8, :], mem], axis=0).astype(BF)
        h = jnp.concatenate([xs[0:16, :], tail], axis=0)
        NG = HB // G
        st1, st2, st3, st4 = {}, {}, {}, {}
        acc = jnp.zeros((SEG, D_), F32)

        def s1(g):
            out = []
            for hd in range(g * G, (g + 1) * G):
                w = pltpu.bitcast(w3[hd], BF)
                qkv = _nn(h, w)
                late = ql_ref[hd, pl.ds(l0, MEM), :].astype(F32)
                q = qkv[:, 0:128] * bscale
                k = qkv[:, 128:256]
                v = qkv[:, 256:384]
                parts = []
                for t, a in enumerate((q, k, v)):
                    rows = [a[0:NE], late[:, t * 128:(t + 1) * 128], a[NE:SEG]]
                    if F32ATT:
                        parts.append(jnp.concatenate(rows, axis=0))
                    else:
                        parts.append(jnp.concatenate(rows + [z8], axis=0).astype(BF))
                out.append(tuple(parts))
            st1[g] = out

        def s2(g):
            out = []
            for (q, k, v) in st1.pop(g):
                sc = _nt(q, k)
                sc = jnp.where(keep, sc, fill)
                mx = jnp.max(sc, axis=1, keepdims=True)
                out.append((sc, mx, v))
            st2[g] = out

        def s3(g):
            out = []
            for (sc, mx, v) in st2.pop(g):
                e = jnp.exp2(sc - mx)
                l = jnp.sum(e, axis=1, keepdims=True)
                out.append((e if F32ATT else e.astype(BF), l, v))
            st3[g] = out

        def s4(g):
            out = []
            for (e, l, v) in st3.pop(g):
                o = _nn(e, v)
                r = pltpu.reciprocal(l, approx=True)
                r = r * (2.0 - l * r)
                out.append((o, r))
            st4[g] = out

        def s5(g, acc):
            for hl, (o, r) in enumerate(st4.pop(g)):
                hd = g * G + hl
                on = o * r
                ol_ref[pl.ds(l0, MEM), hd * 128:(hd + 1) * 128] = on[NE:SEG].astype(BF)
                oc = jnp.concatenate([on[0:NE], on[SEG:SEG + MEM]], axis=0).astype(BF)
                wo_h = pltpu.bitcast(wo2[hd], BF)
                acc = acc + _nn(oc, wo_h)
            return acc

        for t in range(NG + 4):
            if t < NG:
                s1(t)
            if 0 <= t - 1 < NG:
                s2(t - 1)
            if 0 <= t - 2 < NG:
                s3(t - 2)
            if 0 <= t - 3 < NG:
                s4(t - 3)
            if 0 <= t - 4 < NG:
                acc = s5(t - 4, acc)
        b = acc[0:NE, :]
        om = omg_ref[pl.ds(r0, NE), :]
        omt = jnp.concatenate([om] * 4, axis=1)
        o_ref[pl.ds(r0, NE), :] = (ga_ref[pl.ds(r0, NE), :] + omt * b).astype(o_ref.dtype)
        return acc[NE:SEG, :].astype(BF).astype(F32)

    with jax.named_scope("B"):
        lax.fori_loop(0, NSEG, b_step, mem0_ref[...].astype(F32))

    with jax.named_scope("BL2"):
        bl = jnp.zeros((NL, D_), F32)
        for hd in range(HB):
            bl = bl + _nn(ol_ref[:, hd * 128:(hd + 1) * 128], pltpu.bitcast(wo2[hd], BF))
        bl_ref[...] = bl
        for s in range(NSEG):
            rows = slice(s * SEG + NE, (s + 1) * SEG)
            om = omg_ref[rows, :]
            omt = jnp.concatenate([om] * 4, axis=1)
            o_ref[rows, :] = (ga_ref[rows, :] + omt * bl_ref[s * MEM:(s + 1) * MEM, :]).astype(o_ref.dtype)


def pallas_gated_mix__mha_block__memory_aug_recurrent_mem_tr__prompt_kernel(
        A_x, A_wqkv, A_wo, B_x, B_mem0, B_Wq, B_Wk, B_Wv, B_Wo, B_seg_len, gate_w):
    del B_x
    assert B_seg_len == SEG
    x = A_x.reshape(S_, D_)
    mem0 = B_mem0.reshape(MEM, D_)
    gw = gate_w.reshape(1, D_)
    wq = B_Wq.reshape(NCH, D_ * HB // NCH, DB)
    wk = B_Wk.reshape(NCH, D_ * HB // NCH, DB)
    wv = B_Wv.reshape(NCH, D_ * HB // NCH, DB)
    vm = pl.BlockSpec(memory_space=pltpu.VMEM)
    hbm = pl.BlockSpec(memory_space=pl.ANY)
    out = pl.pallas_call(
        _kernel,
        out_shape=jax.ShapeDtypeStruct((S_, D_), A_x.dtype),
        in_specs=[vm, vm, vm, vm, vm, hbm, hbm, hbm, hbm],
        out_specs=vm,
        scratch_shapes=[
            pltpu.VMEM((NCH, D_ * HB // NCH, DB), BF),
            pltpu.VMEM((NCH, D_ * HB // NCH, DB), BF),
            pltpu.VMEM((NCH, D_ * HB // NCH, DB), BF),
            pltpu.VMEM((HB, DB, D_), BF),
            pltpu.VMEM((HB, D_ // 2, 3 * DB), U32),
            pltpu.VMEM((HB, DB // 2, D_), U32),
            pltpu.VMEM((NQB, D_, QB), BF),
            pltpu.VMEM((4, S_ // 2, 128), U32),
            pltpu.VMEM((NQB, D_, QB), BF),
            pltpu.VMEM((NQB, D_, QB), BF),
            pltpu.VMEM((S_, D_), F32),
            pltpu.VMEM((S_, 128), F32),
            pltpu.VMEM((S_, QB), F32),
            pltpu.VMEM((S_, QB), F32),
            pltpu.VMEM((S_ // 2, 128), U32),
            pltpu.VMEM((NSEG * MEM, D_), BF),
            pltpu.VMEM((HB, NSEG * MEM, 3 * DB), BF),
            pltpu.VMEM((NSEG * MEM, HB * DB), BF),
            pltpu.VMEM((NSEG * MEM, D_), F32),
            pltpu.VMEM((1, QB), F32),
            pltpu.SemaphoreType.DMA((4,)),
        ],
        compiler_params=pltpu.CompilerParams(vmem_limit_bytes=100 * 1024 * 1024),
    )(x, A_wqkv, A_wo, mem0, gw, wq, wk, wv, B_Wo)
    return out.reshape(1, S_, D_)
```

```python
import functools
import math

import jax
import jax.numpy as jnp
import numpy as np
from jax import lax
from jax.experimental import pallas as pl
from jax.experimental.pallas import tpu as pltpu

BF = jnp.bfloat16
F32 = jnp.float32
U32 = jnp.uint32
LOG2E = math.log2(math.e)

S_, D_ = 2048, 512
HA, DA = 32, 16
HB, DB = 32, 128
MEM, SEG = 8, 32
NSEG = S_ // SEG
QB = 512
NQB = S_ // QB
LAG = 1
BOFF = 0
SUMMODE = 1
UL = 4
KC = 128
G = 2
NCH = 32


def _nn(a, b):
    return lax.dot_general(a, b, (((1,), (0,)), ((), ())), preferred_element_type=F32)


def _nt(a, b):
    return lax.dot_general(a, b, (((1,), (1,)), ((), ())), preferred_element_type=F32)


def _tn(a, b):
    return lax.dot_general(a, b, (((0,), (0,)), ((), ())), preferred_element_type=F32)


def _kernel(x_hbm, wqkv_hbm, wo_hbm, mem0_ref, gw_ref,
            wq_hbm, wk_hbm, wv_hbm, wo2_hbm,
            o_hbm,
            x_ref, wqkv_ref, wo_ref, o_ref,
            st_q, st_k, st_v, st_o, w3, wo2, qt_ref, kc_ref, vt_ref, ot_ref,
            b_ref, omg_ref, s_a, s_b, kr_ref, xl_ref, ql_ref, ol_ref, bl_ref,
            sems, xsems, osems):
    def x_copy(qb):
        return pltpu.make_async_copy(
            x_hbm.at[pl.ds(qb * QB, QB), :], x_ref.at[pl.ds(qb * QB, QB), :], xsems.at[qb])

    def o_copy(qb):
        return pltpu.make_async_copy(
            o_ref.at[pl.ds(qb * QB, QB), :], o_hbm.at[pl.ds(qb * QB, QB), :], osems.at[qb])

    wqkv_copy = pltpu.make_async_copy(wqkv_hbm, wqkv_ref, sems.at[4])
    wo_copy = pltpu.make_async_copy(wo_hbm, wo_ref, sems.at[5])
    copies = [
        pltpu.make_async_copy(wq_hbm, st_q, sems.at[0]),
        pltpu.make_async_copy(wk_hbm, st_k, sems.at[1]),
        pltpu.make_async_copy(wv_hbm, st_v, sems.at[2]),
        pltpu.make_async_copy(wo2_hbm, st_o, sems.at[3]),
    ]
    wqkv_copy.start()
    x_copy(0).start()
    wqkv_copy.wait()
    x_copy(0).wait()
    for qb in range(1, NQB):
        x_copy(qb).start()
    copies[0].start()

    qscale = (DA ** -0.5) * LOG2E
    wq = wqkv_ref[:, 0:D_]
    wk = wqkv_ref[:, D_:2 * D_]
    wv = wqkv_ref[:, 2 * D_:3 * D_]
    def a0_block(qb, carry):
        r0 = pl.multiple_of(qb * QB, QB)
        @pl.when(qb > 0)
        def _():
            pltpu.make_async_copy(
                x_hbm.at[pl.ds(r0, QB), :], x_ref.at[pl.ds(r0, QB), :], xsems.at[qb]).wait()

        @pl.when(qb == 1)
        def _():
            copies[1].start()

        @pl.when(qb == 2)
        def _():
            copies[2].start()

        @pl.when(qb == 3)
        def _():
            copies[3].start()
            wo_copy.start()

        xb = x_ref[pl.ds(r0, QB), :]
        kk = _nn(xb, wk).astype(BF)
        for g in range(4):
            kc_ref[g, pl.ds(pl.multiple_of(qb * (QB // 2), QB // 2), QB // 2), :] = pltpu.bitcast(kk[:, g * 128:(g + 1) * 128], U32)
        qT = lax.dot_general(wq, xb, (((0,), (1,)), ((), ())),
                             preferred_element_type=F32)
        qt_ref[qb] = (qT * qscale).astype(BF)
        vT = lax.dot_general(wv, xb, (((0,), (1,)), ((), ())),
                             preferred_element_type=F32)
        vt_ref[qb] = vT.astype(BF)
        xf = xb.astype(F32)
        gl = jnp.sum(xf * gw_ref[...].astype(F32), axis=1, keepdims=True)
        gate = 1.0 / (1.0 + jnp.exp(-gl))
        omg_ref[pl.ds(r0, QB), :] = jnp.broadcast_to(gate, (QB, 128))
        return carry

    with jax.named_scope("A0"):
        lax.fori_loop(0, NQB, a0_block, 0)


    NKC = S_ // KC
    NU = HA * NQB
    sbufs = (s_a, s_b)

    def krol_store(hn, c):
        hn = jnp.minimum(hn, HA - 1)
        g = hn // 8
        j = hn % 8
        rows = slice(c * (KC // 2), (c + 1) * (KC // 2))
        kr_ref[rows, :] = pltpu.roll(kc_ref[g, rows, :], (128 - DA * j) % 128, 1)

    def a_s1(qh, sbuf, kc, mrun):
        kr = pltpu.bitcast(kr_ref[kc * (KC // 2):(kc + 1) * (KC // 2), :], BF)
        sT = _nn(kr[:, 0:DA], qh)
        sbuf[kc * KC:(kc + 1) * KC, :] = sT
        mp = jnp.max(sT.reshape(KC // 8, 8, QB), axis=0)
        return mp if mrun is None else jnp.maximum(mrun, mp)

    def a_s2(h, sbuf, kc, m, acc, lneg):
        sT = sbuf[kc * KC:(kc + 1) * KC, :]
        e = jnp.exp2(sT - m)
        parts = []
        for r in range(KC // 32 - 1, -1, -1):
            e0, e1, e2, e3 = [e[r * 32 + 8 * i:r * 32 + 8 * i + 8, :] for i in range(4)]
            t = (e0 + e1) + (e2 + e3)
            lneg = -t if lneg is None else lneg - t
            parts.append(jnp.concatenate([jnp.maximum(e0, lneg), e1, e2, e3], axis=0))
        p = jnp.concatenate(parts[::-1], axis=0).astype(BF)
        vt = vt_ref[kc // (QB // KC), pl.ds(pl.multiple_of(h * DA, DA), DA), (kc % (QB // KC)) * KC:(kc % (QB // KC) + 1) * KC]
        d = _nn(vt, p)
        return (d if acc is None else acc + d), lneg

    def a_fin(h, qb, acc, lneg):
        l = -jnp.sum(lneg, axis=0, keepdims=True)
        r = pltpu.reciprocal(l, approx=True)
        r = r * (2.0 - l * r)
        o = acc * r
        ot_ref[qb, pl.ds(pl.multiple_of(h * DA, DA), DA), :] = o.astype(BF)

    def a_units(h, hpy, state, extra=None):
        acc, lneg, m1, m2 = state
        for qb in range(NQB):
            pi = hpy * NQB + qb
            do1 = pi < NU
            if do1:
                qh = qt_ref[qb, pl.ds(pl.multiple_of(h * DA, DA), DA), :]
            mrun = None
            for c in range(NKC):
                if do1:
                    mrun = a_s1(qh, sbufs[pi % 2], c, mrun)
                    if qb == NQB - 1 and hpy < HA - 1:
                        krol_store(h + 1, c)
                if c < LAG:
                    back, c2, mm = 2, NKC - LAG + c, m2
                else:
                    back, c2, mm = 1, c - LAG, m1
                p2 = pi - back
                if 0 <= p2 < NU:
                    qb2 = qb - back
                    h2 = h if qb2 >= 0 else h - 1
                    qb2 = qb2 % NQB
                    if c2 == 0:
                        acc, lneg = None, None
                    acc, lneg = a_s2(h2, sbufs[p2 % 2], c2, mm, acc, lneg)
                    if c2 == NKC - 1:
                        a_fin(h2, qb2, acc, lneg)
                if extra is not None:
                    extra(qb * NKC + c)
            m2 = m1
            m1 = jnp.max(mrun, axis=0, keepdims=True) if do1 else None
            if not do1 and pi >= NU + 1:
                break
        return acc, lneg, m1, m2

    CH = 256 // NCH

    sub_i = lax.broadcasted_iota(jnp.int32, (8, 128), 0)

    def relayout_w(ci, t):
        w32 = (st_q, st_k, st_v)[t].at[ci].bitcast(U32)
        cur = []
        for T in range(32):
            if T <= 24:
                cur.append(w32[pl.ds(T, 8, stride=33), :])
            else:
                n1 = 32 - T
                cur.append(jnp.concatenate(
                    [w32[pl.ds(T, n1, stride=33), :], w32[pl.ds(32 * n1, 8 - n1, stride=33), :]], axis=0))
        for k in range(3):
            bit = ((sub_i >> k) & 1) == 1
            cur = [jnp.where(bit, cur[(x - (1 << k)) % 32], cur[x]) for x in range(32)]
        ob = pl.multiple_of(ci * CH, CH)
        for j in range(16):
            a, b = cur[j], cur[16 + j]
            w3[2 * j, pl.ds(ob, CH), t * 128:(t + 1) * 128] = (a & U32(0xFFFF)) | (b << 16)
            w3[2 * j + 1, pl.ds(ob, CH), t * 128:(t + 1) * 128] = (a >> 16) | (b & U32(0xFFFF0000))

    bscale = (DB ** -0.5) * LOG2E
    NE = SEG - MEM
    NL = NSEG * MEM
    LP = SEG + MEM
    ri = lax.broadcasted_iota(jnp.int32, (LP, LP), 0)
    ci_ = lax.broadcasted_iota(jnp.int32, (LP, LP), 1)
    keep = (ri >= SEG) | (ci_ >= SEG) | (ci_ <= ri)
    NG = HB // G
    NBS = NG + 4

    class BStep:
        def __init__(self, s, mem):
            r0 = pl.multiple_of(s * SEG, SEG)
            self.r0 = r0
            self.l0 = pl.multiple_of(s * MEM, MEM)
            xs = x_ref[pl.ds(r0, SEG), :]
            tail = jnp.concatenate([xs[16:SEG, :].astype(F32)[0:8, :], mem], axis=0).astype(BF)
            self.h = jnp.concatenate([xs[0:16, :], tail], axis=0)
            self.st1, self.st2, self.st3, self.st4 = {}, {}, {}, {}
            self.acc = None

        def s1(self, g):
            out = []
            for hd in range(g * G, (g + 1) * G):
                w = pltpu.bitcast(w3[hd], BF)
                qkv = _nn(self.h, w)
                late = [ql_ref[t, hd, pl.ds(self.l0, MEM), :].astype(F32) for t in range(3)]
                q = qkv[:, 0:128] * bscale
                k = qkv[:, 128:256]
                v = qkv[:, 256:384]
                out.append(tuple(
                    jnp.concatenate([a[0:NE], late[t], a[NE:SEG]], axis=0)
                    for t, a in enumerate((q, k, v))))
            self.st1[g] = out

        def s2(self, g):
            out = []
            for (q, k, v) in self.st1.pop(g):
                sc = _nt(q, k)
                sc = jnp.where(keep, sc, -1e9 * LOG2E)
                mx = jnp.max(sc, axis=1, keepdims=True)
                out.append((sc, mx, v))
            self.st2[g] = out

        def s3(self, g):
            out = []
            for (sc, mx, v) in self.st2.pop(g):
                e = jnp.exp2(sc - mx)
                l = jnp.sum(e, axis=1, keepdims=True)
                out.append((e, l, v))
            self.st3[g] = out

        def s4(self, g):
            out = []
            for (e, l, v) in self.st3.pop(g):
                o = _nn(e, v)
                r = pltpu.reciprocal(l, approx=True)
                r = r * (2.0 - l * r)
                out.append((o, r))
            self.st4[g] = out

        def s5(self, g):
            for hl, (o, r) in enumerate(self.st4.pop(g)):
                hd = g * G + hl
                on = o * r
                ol_ref[pl.ds(self.l0, MEM), hd * 128:(hd + 1) * 128] = on[NE:SEG].astype(BF)
                oc = jnp.concatenate([on[0:NE], on[SEG:SEG + MEM]], axis=0).astype(BF)
                d = _nn(oc, pltpu.bitcast(wo2[hd], BF))
                self.acc = d if self.acc is None else self.acc + d

        def slot(self, t):
            if t < NG:
                self.s1(t)
            if 0 <= t - 1 < NG:
                self.s2(t - 1)
            if 0 <= t - 2 < NG:
                self.s3(t - 2)
            if 0 <= t - 3 < NG:
                self.s4(t - 3)
            if 0 <= t - 4 < NG:
                self.s5(t - 4)

        def finish(self):
            b_ref[pl.ds(self.r0, NE), :] = self.acc[0:NE, :]
            return self.acc[NE:SEG, :].astype(BF).astype(F32)

    class BTwo:
        def __init__(self, s0, mem):
            self.s0, self.mem, self.k, self.cur = s0, mem, 0, None

        def emit(self):
            if self.k >= 2 * NBS:
                return
            step, t = divmod(self.k, NBS)
            if t == 0:
                self.cur = BStep(self.s0 + step, self.mem)
            self.cur.slot(t)
            if t == NBS - 1:
                self.mem = self.cur.finish()
            self.k += 1

        def upto(self, n):
            while self.k < min(n, 2 * NBS):
                self.emit()

    with jax.named_scope("A1a"):
        for c in range(NKC):
            krol_store(0, c)
        st = a_units(0, 0, (None, None, None, None))

    with jax.named_scope("BL1"):
        for s in range(NSEG):
            xl_ref[s * MEM:(s + 1) * MEM, :] = x_ref[s * SEG + NE:(s + 1) * SEG, :]

        for t in range(3):
            copies[t].wait()

            def relayout(ci, carry, t=t):
                relayout_w(ci, t)
                return carry

            lax.fori_loop(0, NCH, relayout, 0)

            def bl1(i, carry, t=t):
                for u in range(UL):
                    hd0 = (i * UL + u) * 4
                    w = jnp.concatenate(
                        [pltpu.bitcast(w3[hd0 + n, :, t * 128:(t + 1) * 128], BF) for n in range(4)], axis=1)
                    r = _nn(xl_ref[...], w)
                    if t == 0:
                        r = r * bscale
                    r = r.astype(BF)
                    for n in range(4):
                        ql_ref[t, hd0 + n] = r[:, n * 128:(n + 1) * 128]
                return carry

            lax.fori_loop(0, HB // (4 * UL), bl1, 0)

        copies[3].wait()

        def relayout_o(ci, carry):
            wo2[ci] = pltpu.bitcast(st_o[ci], U32)
            return carry

        lax.fori_loop(0, HB, relayout_o, 0)

    with jax.named_scope("main"):
        NSLOT = NQB * NKC

        def body(i, carry):
            st, mem = carry
            bt = BTwo(2 * (i - 1), mem)
            st = a_units(i, 1, st, extra=lambda slot: bt.upto(((slot + 1) * 2 * NBS + BOFF) // NSLOT))
            bt.upto(2 * NBS)
            return st, bt.mem

        st, mem = lax.fori_loop(1, HA, body, (st, mem0_ref[...].astype(F32)))
        bt = BTwo(2 * (HA - 1), mem)
        a_units(HA, HA, st, extra=lambda slot: bt.upto(slot + 1))
        bt.upto(2 * NBS)

    with jax.named_scope("BL2"):
        bl = None
        for hd in range(HB):
            d = _nn(ol_ref[:, hd * 128:(hd + 1) * 128], pltpu.bitcast(wo2[hd], BF))
            bl = d if bl is None else bl + d
        bl_ref[...] = bl
        for s in range(NSEG):
            b_ref[s * SEG + NE:(s + 1) * SEG, :] = bl_ref[s * MEM:(s + 1) * MEM, :]

    with jax.named_scope("final"):
        wo_copy.wait()
        for qb in range(NQB):
            rows = slice(qb * QB, (qb + 1) * QB)
            a = _tn(ot_ref[qb], wo_ref[...])
            gate = omg_ref[rows, :]
            gt = jnp.concatenate([gate] * 4, axis=1)
            o_ref[rows, :] = (gt * a + (1.0 - gt) * b_ref[rows, :]).astype(o_ref.dtype)
            o_copy(qb).start()
        for qb in range(NQB):
            o_copy(qb).wait()


def pallas_gated_mix__mha_block__memory_aug_recurrent_mem_tr__prompt_kernel(
        A_x, A_wqkv, A_wo, B_x, B_mem0, B_Wq, B_Wk, B_Wv, B_Wo, B_seg_len, gate_w):
    del B_x
    assert B_seg_len == SEG
    x = A_x.reshape(S_, D_)
    mem0 = B_mem0.reshape(MEM, D_)
    gw = gate_w.reshape(1, D_)
    wq = B_Wq.reshape(NCH, D_ * HB // NCH, DB)
    wk = B_Wk.reshape(NCH, D_ * HB // NCH, DB)
    wv = B_Wv.reshape(NCH, D_ * HB // NCH, DB)
    vm = pl.BlockSpec(memory_space=pltpu.VMEM)
    hbm = pl.BlockSpec(memory_space=pl.ANY)
    out = pl.pallas_call(
        _kernel,
        out_shape=jax.ShapeDtypeStruct((S_, D_), A_x.dtype),
        in_specs=[hbm, hbm, hbm, vm, vm, hbm, hbm, hbm, hbm],
        out_specs=hbm,
        scratch_shapes=[
            pltpu.VMEM((S_, D_), BF),
            pltpu.VMEM((D_, 3 * D_), BF),
            pltpu.VMEM((D_, D_), BF),
            pltpu.VMEM((S_, D_), BF),
            pltpu.VMEM((NCH, D_ * HB // NCH, DB), BF),
            pltpu.VMEM((NCH, D_ * HB // NCH, DB), BF),
            pltpu.VMEM((NCH, D_ * HB // NCH, DB), BF),
            pltpu.VMEM((HB, DB, D_), BF),
            pltpu.VMEM((HB, D_ // 2, 3 * DB), U32),
            pltpu.VMEM((HB, DB // 2, D_), U32),
            pltpu.VMEM((NQB, D_, QB), BF),
            pltpu.VMEM((4, S_ // 2, 128), U32),
            pltpu.VMEM((NQB, D_, QB), BF),
            pltpu.VMEM((NQB, D_, QB), BF),
            pltpu.VMEM((S_, D_), F32),
            pltpu.VMEM((S_, 128), F32),
            pltpu.VMEM((S_, QB), F32),
            pltpu.VMEM((S_, QB), F32),
            pltpu.VMEM((S_ // 2, 128), U32),
            pltpu.VMEM((NSEG * MEM, D_), BF),
            pltpu.VMEM((3, HB, NSEG * MEM, DB), BF),
            pltpu.VMEM((NSEG * MEM, HB * DB), BF),
            pltpu.VMEM((NSEG * MEM, D_), F32),
            pltpu.SemaphoreType.DMA((6,)),
            pltpu.SemaphoreType.DMA((NQB,)),
            pltpu.SemaphoreType.DMA((NQB,)),
        ],
        compiler_params=pltpu.CompilerParams(vmem_limit_bytes=100 * 1024 * 1024),
    )(x, A_wqkv, A_wo, mem0, gw, wq, wk, wv, B_Wo)
    return out.reshape(1, S_, D_)
```

```python
import math

import jax
import jax.numpy as jnp
import numpy as np
from jax import lax
from jax.experimental import pallas as pl
from jax.experimental.pallas import tpu as pltpu

BF = jnp.bfloat16
F32 = jnp.float32
U32 = jnp.uint32
LOG2E = math.log2(math.e)

S_, D_ = 2048, 512
HA, DA = 32, 16
HB, DB = 32, 128
MEM, SEG = 8, 32
NSEG = S_ // SEG
QB = 512
NQB = S_ // QB
HPB = 1
EVEN = 1
HIDE = 1
LAG = 1
BOFF = 0
SUMMODE = 1
UL = 4
KC = 128
G = 2
NCH = 32


def _nn(a, b):
    return lax.dot_general(a, b, (((1,), (0,)), ((), ())), preferred_element_type=F32)


def _nt(a, b):
    return lax.dot_general(a, b, (((1,), (1,)), ((), ())), preferred_element_type=F32)


def _tn(a, b):
    return lax.dot_general(a, b, (((0,), (0,)), ((), ())), preferred_element_type=F32)


def _kernel(x_hbm, wqkv_hbm, wo_hbm, mem0_ref, gw_ref,
            wq_hbm, wk_hbm, wv_hbm, wo2_hbm,
            o_hbm,
            x_ref, wqkv_ref, wo_ref, o_ref,
            st_q, st_k, st_v, st_o, w3, wo2, qt_ref, kc_ref, vt_ref, ot_ref,
            b_ref, omg_ref, s_a, s_b, kr_ref, xl_ref, ql_ref, ol_ref, bl_ref,
            sems, xsems, osems):
    def x_copy(qb):
        return pltpu.make_async_copy(
            x_hbm.at[pl.ds(qb * QB, QB), :], x_ref.at[pl.ds(qb * QB, QB), :], xsems.at[qb])

    def o_copy(qb):
        return pltpu.make_async_copy(
            o_ref.at[pl.ds(qb * QB, QB), :], o_hbm.at[pl.ds(qb * QB, QB), :], osems.at[qb])

    def wqkv_part(t):
        return pltpu.make_async_copy(
            wqkv_hbm.at[:, pl.ds(t * D_, D_)], wqkv_ref.at[:, pl.ds(t * D_, D_)], sems.at[6 + t])

    wo_copy = pltpu.make_async_copy(wo_hbm, wo_ref, sems.at[5])
    copies = [
        pltpu.make_async_copy(wq_hbm, st_q, sems.at[0]),
        pltpu.make_async_copy(wk_hbm, st_k, sems.at[1]),
        pltpu.make_async_copy(wv_hbm, st_v, sems.at[2]),
        pltpu.make_async_copy(wo2_hbm, st_o, sems.at[3]),
    ]
    x_copy(0).start()
    wqkv_part(1).start()
    x_copy(0).wait()
    wqkv_part(1).wait()
    wqkv_part(0).start()
    wqkv_part(2).start()

    qscale = (DA ** -0.5) * LOG2E

    def a0_block(qb, first):
        r0 = qb * QB if first else pl.multiple_of(qb * QB, QB)
        k0 = qb * (QB // 2) if first else pl.multiple_of(qb * (QB // 2), QB // 2)
        xb = x_ref[pl.ds(r0, QB), :]
        kk = _nn(xb, wqkv_ref[:, D_:2 * D_]).astype(BF)
        for g in range(4):
            kc_ref[g, pl.ds(k0, QB // 2), :] = pltpu.bitcast(kk[:, g * 128:(g + 1) * 128], U32)
        if first:
            wqkv_part(0).wait()
            wqkv_part(2).wait()
            x_copy(1).start()
            copies[0].start()
        qT = lax.dot_general(wqkv_ref[:, 0:D_], xb, (((0,), (1,)), ((), ())),
                             preferred_element_type=F32)
        qt_ref[qb] = (qT * qscale).astype(BF)
        vT = lax.dot_general(wqkv_ref[:, 2 * D_:3 * D_], xb, (((0,), (1,)), ((), ())),
                             preferred_element_type=F32)
        vt_ref[qb] = vT.astype(BF)
        xf = xb.astype(F32)
        gl = jnp.sum(xf * gw_ref[...].astype(F32)[None, :], axis=1, keepdims=True)
        gate = 1.0 / (1.0 + jnp.exp(-gl))
        omg_ref[pl.ds(r0, QB), :] = jnp.broadcast_to(gate, (QB, 128))

    def a0_body(qb, carry):
        r0 = pl.multiple_of(qb * QB, QB)
        pltpu.make_async_copy(
            x_hbm.at[pl.ds(r0, QB), :], x_ref.at[pl.ds(r0, QB), :], xsems.at[qb]).wait()

        @pl.when(qb == 1)
        def _():
            x_copy(2).start()
            x_copy(3).start()
            copies[1].start()

        @pl.when(qb == 2)
        def _():
            copies[2].start()

        @pl.when(qb == 3)
        def _():
            copies[3].start()
            wo_copy.start()

        a0_block(qb, False)
        return carry

    with jax.named_scope("A0"):
        a0_block(0, True)
        lax.fori_loop(1, NQB, a0_body, 0)


    NKC = S_ // KC
    NU = HA * NQB
    sbufs = (s_a, s_b)

    def krol_store(hn, c):
        hn = jnp.minimum(hn, HA - 1)
        g = hn // 8
        j = hn % 8
        rows = slice(c * (KC // 2), (c + 1) * (KC // 2))
        kr_ref[rows, :] = pltpu.roll(kc_ref[g, rows, :], (128 - DA * j) % 128, 1)

    def a_s1(qh, sbuf, kc, mrun):
        kr = pltpu.bitcast(kr_ref[kc * (KC // 2):(kc + 1) * (KC // 2), :], BF)
        sT = _nn(kr[:, 0:DA], qh)
        sbuf[kc * KC:(kc + 1) * KC, :] = sT
        mp = jnp.max(sT.reshape(KC // 8, 8, QB), axis=0)
        return mp if mrun is None else jnp.maximum(mrun, mp)

    def a_s2(h, sbuf, kc, m, acc, lneg):
        sT = sbuf[kc * KC:(kc + 1) * KC, :]
        e = jnp.exp2(sT - m)
        parts = []
        for r in range(KC // 32 - 1, -1, -1):
            e0, e1, e2, e3 = [e[r * 32 + 8 * i:r * 32 + 8 * i + 8, :] for i in range(4)]
            t = (e0 + e1) + (e2 + e3)
            lneg = -t if lneg is None else lneg - t
            parts.append(jnp.concatenate([jnp.maximum(e0, lneg), e1, e2, e3], axis=0))
        p = jnp.concatenate(parts[::-1], axis=0).astype(BF)
        vt = vt_ref[kc // (QB // KC), pl.ds(pl.multiple_of(h * DA, DA), DA), (kc % (QB // KC)) * KC:(kc % (QB // KC) + 1) * KC]
        d = _nn(vt, p)
        return (d if acc is None else acc + d), lneg

    def a_fin(h, qb, acc, lneg):
        l = -jnp.sum(lneg, axis=0, keepdims=True)
        r = pltpu.reciprocal(l, approx=True)
        r = r * (2.0 - l * r)
        o = acc * r
        ot_ref[qb, pl.ds(pl.multiple_of(h * DA, DA), DA), :] = o.astype(BF)

    def a_units(h, hpy, state, extra=None):
        acc, lneg, m1, m2 = state
        for qb in range(NQB):
            pi = hpy * NQB + qb
            do1 = pi < NU
            if do1:
                qh = qt_ref[qb, pl.ds(pl.multiple_of(h * DA, DA), DA), :]
            mrun = None
            for c in range(NKC):
                if do1:
                    mrun = a_s1(qh, sbufs[pi % 2], c, mrun)
                    if qb == NQB - 1 and hpy < HA - 1:
                        krol_store(h + 1, c)
                if c < LAG:
                    back, c2, mm = 2, NKC - LAG + c, m2
                else:
                    back, c2, mm = 1, c - LAG, m1
                p2 = pi - back
                if 0 <= p2 < NU:
                    qb2 = qb - back
                    h2 = h if qb2 >= 0 else h - 1
                    qb2 = qb2 % NQB
                    if c2 == 0:
                        acc, lneg = None, None
                    acc, lneg = a_s2(h2, sbufs[p2 % 2], c2, mm, acc, lneg)
                    if c2 == NKC - 1:
                        a_fin(h2, qb2, acc, lneg)
                if extra is not None:
                    extra(qb * NKC + c)
            m2 = m1
            m1 = jnp.max(mrun, axis=0, keepdims=True) if do1 else None
            if not do1 and pi >= NU + 1:
                break
        return acc, lneg, m1, m2

    CH = 256 // NCH

    sub_i = lax.broadcasted_iota(jnp.int32, (8, 128), 0)

    def relayout_w(ci, t):
        w32 = (st_q, st_k, st_v)[t].at[ci].bitcast(U32)
        cur = []
        for T in range(32):
            if T <= 24:
                cur.append(w32[pl.ds(T, 8, stride=33), :])
            else:
                n1 = 32 - T
                cur.append(jnp.concatenate(
                    [w32[pl.ds(T, n1, stride=33), :], w32[pl.ds(32 * n1, 8 - n1, stride=33), :]], axis=0))
        for k in range(3):
            bit = ((sub_i >> k) & 1) == 1
            cur = [jnp.where(bit, cur[(x - (1 << k)) % 32], cur[x]) for x in range(32)]
        ob = pl.multiple_of(ci * CH, CH)
        for j in range(16):
            a, b = cur[j], cur[16 + j]
            w3[2 * j, pl.ds(ob, CH), t * 128:(t + 1) * 128] = (a & U32(0xFFFF)) | (b << 16)
            w3[2 * j + 1, pl.ds(ob, CH), t * 128:(t + 1) * 128] = (a >> 16) | (b & U32(0xFFFF0000))

    bscale = (DB ** -0.5) * LOG2E
    NE = SEG - MEM
    NL = NSEG * MEM
    LP = SEG + MEM
    ri = lax.broadcasted_iota(jnp.int32, (LP, LP), 0)
    ci_ = lax.broadcasted_iota(jnp.int32, (LP, LP), 1)
    keep = (ri >= SEG) | (ci_ >= SEG) | (ci_ <= ri)
    NG = HB // G
    NBS = NG + 4

    class BStep:
        def __init__(self, s, mem):
            r0 = pl.multiple_of(s * SEG, SEG)
            self.r0 = r0
            self.l0 = pl.multiple_of(s * MEM, MEM)
            xs = x_ref[pl.ds(r0, SEG), :]
            tail = jnp.concatenate([xs[16:SEG, :].astype(F32)[0:8, :], mem], axis=0).astype(BF)
            self.h = jnp.concatenate([xs[0:16, :], tail], axis=0)
            self.st1, self.st2, self.st3, self.st4 = {}, {}, {}, {}
            self.acc = None

        def s1(self, g):
            out = []
            for hd in range(g * G, (g + 1) * G):
                w = pltpu.bitcast(w3[hd], BF)
                qkv = _nn(self.h, w)
                late = [ql_ref[t, hd, pl.ds(self.l0, MEM), :].astype(F32) for t in range(3)]
                q = qkv[:, 0:128] * bscale
                k = qkv[:, 128:256]
                v = qkv[:, 256:384]
                out.append(tuple(
                    jnp.concatenate([a[0:NE], late[t], a[NE:SEG]], axis=0)
                    for t, a in enumerate((q, k, v))))
            self.st1[g] = out

        def s2(self, g):
            out = []
            for (q, k, v) in self.st1.pop(g):
                sc = _nt(q, k)
                sc = jnp.where(keep, sc, -1e9 * LOG2E)
                mx = jnp.max(sc, axis=1, keepdims=True)
                out.append((sc, mx, v))
            self.st2[g] = out

        def s3(self, g):
            out = []
            for (sc, mx, v) in self.st2.pop(g):
                e = jnp.exp2(sc - mx)
                l = jnp.sum(e, axis=1, keepdims=True)
                out.append((e, l, v))
            self.st3[g] = out

        def s4(self, g):
            out = []
            for (e, l, v) in self.st3.pop(g):
                o = _nn(e, v)
                r = pltpu.reciprocal(l, approx=True)
                r = r * (2.0 - l * r)
                out.append((o, r))
            self.st4[g] = out

        def s5(self, g):
            for hl, (o, r) in enumerate(self.st4.pop(g)):
                hd = g * G + hl
                on = o * r
                ol_ref[pl.ds(self.l0, MEM), hd * 128:(hd + 1) * 128] = on[NE:SEG].astype(BF)
                oc = jnp.concatenate([on[0:NE], on[SEG:SEG + MEM]], axis=0).astype(BF)
                d = _nn(oc, pltpu.bitcast(wo2[hd], BF))
                self.acc = d if self.acc is None else self.acc + d

        def slot(self, t):
            if t < NG:
                self.s1(t)
            if 0 <= t - 1 < NG:
                self.s2(t - 1)
            if 0 <= t - 2 < NG:
                self.s3(t - 2)
            if 0 <= t - 3 < NG:
                self.s4(t - 3)
            if 0 <= t - 4 < NG:
                self.s5(t - 4)

        def finish(self):
            b_ref[pl.ds(self.r0, NE), :] = self.acc[0:NE, :]
            return self.acc[NE:SEG, :].astype(BF).astype(F32)

    class BTwo:
        def __init__(self, s0, mem):
            self.s0, self.mem, self.k, self.cur = s0, mem, 0, None

        def emit(self):
            if self.k >= 2 * NBS:
                return
            step, t = divmod(self.k, NBS)
            if t == 0:
                self.cur = BStep(self.s0 + step, self.mem)
            self.cur.slot(t)
            if t == NBS - 1:
                self.mem = self.cur.finish()
            self.k += 1

        def upto(self, n):
            while self.k < min(n, 2 * NBS):
                self.emit()

    def relayout_o(ci):
        wo2[ci] = pltpu.bitcast(st_o[ci], U32)

    with jax.named_scope("A1a"):
        for c in range(NKC):
            krol_store(0, c)

        def pre_extra(slot):
            if slot == 31:
                copies[0].wait()
            if slot >= 32:
                relayout_w(slot - 32, 0)

        st = a_units(0, 0, (None, None, None, None), extra=pre_extra if HIDE else None)

    with jax.named_scope("BL1"):
        for s in range(NSEG):
            xl_ref[s * MEM:(s + 1) * MEM, :] = x_ref[s * SEG + NE:(s + 1) * SEG, :]

        for t in range(3):
            if HIDE:
                copies[t + 1].wait()
            else:
                copies[t].wait()

                def relayout(ci, carry, t=t):
                    relayout_w(ci, t)
                    return carry

                lax.fori_loop(0, NCH, relayout, 0)

            def bl1(i, carry, t=t):
                for u in range(UL):
                    hd0 = (i * UL + u) * 4
                    w = jnp.concatenate(
                        [pltpu.bitcast(w3[hd0 + n, :, t * 128:(t + 1) * 128], BF) for n in range(4)], axis=1)
                    r = _nn(xl_ref[...], w)
                    if t == 0:
                        r = r * bscale
                    r = r.astype(BF)
                    for n in range(4):
                        ql_ref[t, hd0 + n] = r[:, n * 128:(n + 1) * 128]
                    if HIDE:
                        for n in range(4):
                            if t < 2:
                                relayout_w(hd0 + n, t + 1)
                            else:
                                relayout_o(hd0 + n)
                return carry

            lax.fori_loop(0, HB // (4 * UL), bl1, 0)

        if not HIDE:
            copies[3].wait()

            def relayout_o_body(ci, carry):
                relayout_o(ci)
                return carry

            lax.fori_loop(0, HB, relayout_o_body, 0)

    with jax.named_scope("main"):
        NSLOT = NQB * NKC

        def two(h, carry):
            st, mem = carry
            bt = BTwo(2 * (h - 1), mem)
            st = a_units(h, 1, st, extra=lambda slot: bt.upto(((slot + 1) * 2 * NBS + BOFF) // NSLOT))
            bt.upto(2 * NBS)
            return st, bt.mem

        carry = (st, mem0_ref[...].astype(F32))
        if HPB == 1:
            carry = lax.fori_loop(1, HA, two, carry)
        else:
            nit = (HA - 1) // HPB
            def body(i, carry):
                for k in range(HPB):
                    carry = two(1 + i * HPB + k, carry)
                return carry
            carry = lax.fori_loop(0, nit, body, carry)
            for h in range(1 + nit * HPB, HA):
                carry = two(h, carry)
        st, mem = carry
        bt = BTwo(2 * (HA - 1), mem)
        a_units(HA, HA, st, extra=lambda slot: bt.upto(slot + 1))
        bt.upto(2 * NBS)

    with jax.named_scope("BL2"):
        bl = None
        for hd in range(HB):
            d = _nn(ol_ref[:, hd * 128:(hd + 1) * 128], pltpu.bitcast(wo2[hd], BF))
            bl = d if bl is None else bl + d
        bl_ref[...] = bl
        for s in range(NSEG):
            b_ref[s * SEG + NE:(s + 1) * SEG, :] = bl_ref[s * MEM:(s + 1) * MEM, :]

    with jax.named_scope("final"):
        wo_copy.wait()
        for qb in range(NQB):
            rows = slice(qb * QB, (qb + 1) * QB)
            a = _tn(ot_ref[qb], wo_ref[...])
            gate = omg_ref[rows, :]
            gt = jnp.concatenate([gate] * 4, axis=1)
            o_ref[rows, :] = (gt * a + (1.0 - gt) * b_ref[rows, :]).astype(o_ref.dtype)
            o_copy(qb).start()
        for qb in range(NQB):
            o_copy(qb).wait()


def pallas_gated_mix__mha_block__memory_aug_recurrent_mem_tr__prompt_kernel(
        A_x, A_wqkv, A_wo, B_x, B_mem0, B_Wq, B_Wk, B_Wv, B_Wo, B_seg_len, gate_w):
    del B_x
    assert B_seg_len == SEG
    x = A_x.reshape(S_, D_)
    mem0 = B_mem0.reshape(MEM, D_)
    gw = gate_w
    wq = B_Wq.reshape(NCH, D_ * HB // NCH, DB)
    wk = B_Wk.reshape(NCH, D_ * HB // NCH, DB)
    wv = B_Wv.reshape(NCH, D_ * HB // NCH, DB)
    vm = pl.BlockSpec(memory_space=pltpu.VMEM)
    hbm = pl.BlockSpec(memory_space=pl.ANY)
    out = pl.pallas_call(
        _kernel,
        out_shape=jax.ShapeDtypeStruct((S_, D_), A_x.dtype),
        in_specs=[hbm, hbm, hbm, vm, vm, hbm, hbm, hbm, hbm],
        out_specs=hbm,
        scratch_shapes=[
            pltpu.VMEM((S_, D_), BF),
            pltpu.VMEM((D_, 3 * D_), BF),
            pltpu.VMEM((D_, D_), BF),
            pltpu.VMEM((S_, D_), BF),
            pltpu.VMEM((NCH, D_ * HB // NCH, DB), BF),
            pltpu.VMEM((NCH, D_ * HB // NCH, DB), BF),
            pltpu.VMEM((NCH, D_ * HB // NCH, DB), BF),
            pltpu.VMEM((HB, DB, D_), BF),
            pltpu.VMEM((HB, D_ // 2, 3 * DB), U32),
            pltpu.VMEM((HB, DB // 2, D_), U32),
            pltpu.VMEM((NQB, D_, QB), BF),
            pltpu.VMEM((4, S_ // 2, 128), U32),
            pltpu.VMEM((NQB, D_, QB), BF),
            pltpu.VMEM((NQB, D_, QB), BF),
            pltpu.VMEM((S_, D_), F32),
            pltpu.VMEM((S_, 128), F32),
            pltpu.VMEM((S_, QB), F32),
            pltpu.VMEM((S_, QB), F32),
            pltpu.VMEM((S_ // 2, 128), U32),
            pltpu.VMEM((NSEG * MEM, D_), BF),
            pltpu.VMEM((3, HB, NSEG * MEM, DB), BF),
            pltpu.VMEM((NSEG * MEM, HB * DB), BF),
            pltpu.VMEM((NSEG * MEM, D_), F32),
            pltpu.SemaphoreType.DMA((9,)),
            pltpu.SemaphoreType.DMA((NQB,)),
            pltpu.SemaphoreType.DMA((NQB,)),
        ],
        compiler_params=pltpu.CompilerParams(
            vmem_limit_bytes=100 * 1024 * 1024,
            flags={"XLA_TPU_EVENLY_DISTRIBUTE_CRITICAL_NODES": True} if EVEN else None),
    )(x, A_wqkv, A_wo, mem0, gw, wq, wk, wv, B_Wo)
    return out.reshape(1, S_, D_)
```

```python
import math

import jax
import jax.numpy as jnp
from jax import lax
from jax.experimental import pallas as pl
from jax.experimental.pallas import tpu as pltpu

BF = jnp.bfloat16
F32 = jnp.float32
U32 = jnp.uint32
LOG2E = math.log2(math.e)

S_, D_ = 2048, 512
HA, DA = 32, 16
HB, DB = 32, 128
MEM, SEG = 8, 32
NSEG = S_ // SEG
NE = SEG - MEM
NL = NSEG * MEM

QB = 512
NQB = S_ // QB
KC = 128
NKC = S_ // KC
NU = HA * NQB
LAG = 1
GR = 32
G = 2
NG = HB // G
NBS = NG + 4
NCH = 32
CH = D_ // 2 // NCH
UL = 4
FB = 256
NFB = S_ // FB


def _nn(a, b):
    return lax.dot_general(a, b, (((1,), (0,)), ((), ())), preferred_element_type=F32)


def _nt(a, b):
    return lax.dot_general(a, b, (((1,), (1,)), ((), ())), preferred_element_type=F32)


def _tn(a, b):
    return lax.dot_general(a, b, (((0,), (0,)), ((), ())), preferred_element_type=F32)


def _tt(a, b):
    return lax.dot_general(a, b, (((0,), (1,)), ((), ())), preferred_element_type=F32)


def _recip(l):
    r = pltpu.reciprocal(l, approx=True)
    return r * (2.0 - l * r)


def _kernel(x_hbm, wqkv_hbm, wo_hbm, mem0_ref, gw_ref, wq_hbm, wk_hbm, wv_hbm, wo2_hbm,
            o_hbm,
            x_ref, wqkv_ref, wo_ref, o_ref,
            st_q, st_k, st_v, st_o, w3, wo2,
            qt_ref, kc_ref, vt_ref, ot_ref, s_a, s_b, kr_ref, gate_ref,
            xl_ref, ql_ref, ol_ref, bl_ref, b_ref,
            sems, xsems, osems):

    def x_copy(qb):
        return pltpu.make_async_copy(
            x_hbm.at[pl.ds(qb * QB, QB), :], x_ref.at[pl.ds(qb * QB, QB), :], xsems.at[qb])

    def o_copy(fb):
        return pltpu.make_async_copy(
            o_ref.at[pl.ds(fb * FB, FB), :], o_hbm.at[pl.ds(fb * FB, FB), :], osems.at[fb])

    def wqkv_copy(t):
        return pltpu.make_async_copy(
            wqkv_hbm.at[:, pl.ds(t * D_, D_)], wqkv_ref.at[:, pl.ds(t * D_, D_)], sems.at[5 + t])

    wo_copy = pltpu.make_async_copy(wo_hbm, wo_ref, sems.at[4])
    b_copies = [
        pltpu.make_async_copy(wq_hbm, st_q, sems.at[0]),
        pltpu.make_async_copy(wk_hbm, st_k, sems.at[1]),
        pltpu.make_async_copy(wv_hbm, st_v, sems.at[2]),
        pltpu.make_async_copy(wo2_hbm, st_o, sems.at[3]),
    ]
    x_copy(0).start()
    wqkv_copy(1).start()
    x_copy(0).wait()
    wqkv_copy(1).wait()
    wqkv_copy(0).start()
    wqkv_copy(2).start()

    sub_i = lax.broadcasted_iota(jnp.int32, (8, 128), 0)

    def relayout_w(ci, t):
        w32 = (st_q, st_k, st_v)[t].at[ci].bitcast(U32)
        cur = []
        for d in range(32):
            if d <= 24:
                cur.append(w32[pl.ds(d, 8, stride=33), :])
            else:
                n1 = 32 - d
                cur.append(jnp.concatenate(
                    [w32[pl.ds(d, n1, stride=33), :], w32[pl.ds(32 * n1, 8 - n1, stride=33), :]],
                    axis=0))
        for k in range(3):
            bit = ((sub_i >> k) & 1) == 1
            cur = [jnp.where(bit, cur[(x - (1 << k)) % 32], cur[x]) for x in range(32)]
        ob = pl.multiple_of(ci * CH, CH)
        for j in range(16):
            a, b = cur[j], cur[16 + j]
            w3[2 * j, pl.ds(ob, CH), t * 128:(t + 1) * 128] = (a & U32(0xFFFF)) | (b << 16)
            w3[2 * j + 1, pl.ds(ob, CH), t * 128:(t + 1) * 128] = (a >> 16) | (b & U32(0xFFFF0000))

    def relayout_o(hd):
        wo2[hd] = pltpu.bitcast(st_o[hd], U32)

    qscale = (DA ** -0.5) * LOG2E

    def a0_block(qb, first):
        r0 = qb * QB if first else pl.multiple_of(qb * QB, QB)
        k0 = qb * (QB // 2) if first else pl.multiple_of(qb * (QB // 2), QB // 2)
        xb = x_ref[pl.ds(r0, QB), :]
        kk = _nn(xb, wqkv_ref[:, D_:2 * D_]).astype(BF)
        for g in range(4):
            kc_ref[g, pl.ds(k0, QB // 2), :] = pltpu.bitcast(kk[:, g * 128:(g + 1) * 128], U32)
        if first:
            wqkv_copy(0).wait()
            wqkv_copy(2).wait()
            x_copy(1).start()
            b_copies[0].start()
        qt_ref[qb] = (_tt(wqkv_ref[:, 0:D_], xb) * qscale).astype(BF)
        vt_ref[qb] = _tt(wqkv_ref[:, 2 * D_:3 * D_], xb).astype(BF)
        gl = jnp.sum(xb.astype(F32) * gw_ref[...].astype(F32)[None, :], axis=1, keepdims=True)
        gate = 1.0 / (1.0 + jnp.exp(-gl))
        gate_ref[pl.ds(r0, QB), :] = jnp.broadcast_to(gate, (QB, 128))

    def a0_body(qb, carry):
        r0 = pl.multiple_of(qb * QB, QB)
        pltpu.make_async_copy(
            x_hbm.at[pl.ds(r0, QB), :], x_ref.at[pl.ds(r0, QB), :], xsems.at[qb]).wait()

        @pl.when(qb == 1)
        def _():
            x_copy(2).start()
            x_copy(3).start()
            b_copies[1].start()

        @pl.when(qb == 2)
        def _():
            b_copies[2].start()

        @pl.when(qb == 3)
        def _():
            b_copies[3].start()
            wo_copy.start()

        a0_block(qb, False)
        return carry

    a0_block(0, True)
    lax.fori_loop(1, NQB, a0_body, 0)

    sbufs = (s_a, s_b)

    def k_stage(hn, c):
        hn = jnp.minimum(hn, HA - 1)
        rows = slice(c * (KC // 2), (c + 1) * (KC // 2))
        kr_ref[rows, :] = pltpu.roll(kc_ref[hn // 8, rows, :], (128 - DA * (hn % 8)) % 128, 1)

    def a_pass1(qh, sbuf, c, mrun):
        kr = pltpu.bitcast(kr_ref[c * (KC // 2):(c + 1) * (KC // 2), :], BF)
        st = _nn(kr[:, 0:DA], qh)
        sbuf[c * KC:(c + 1) * KC, :] = st
        mp = jnp.max(st.reshape(KC // 8, 8, QB), axis=0)
        return mp if mrun is None else jnp.maximum(mrun, mp)

    def a_pass2(h, sbuf, c, m, acc, lneg):
        e = jnp.exp2(sbuf[c * KC:(c + 1) * KC, :] - m)
        parts = []
        for r in range(KC // GR - 1, -1, -1):
            vs = [e[r * GR + 8 * i:r * GR + 8 * i + 8, :] for i in range(GR // 8)]
            lv = vs
            while len(lv) > 1:
                lv = [lv[2 * i] + lv[2 * i + 1] for i in range(len(lv) // 2)]
            lneg = -lv[0] if lneg is None else lneg - lv[0]
            vs[0] = jnp.maximum(vs[0], lneg)
            parts.append(jnp.concatenate(vs, axis=0))
        p = jnp.concatenate(parts[::-1], axis=0).astype(BF)
        kb, kc = divmod(c, QB // KC)
        vt = vt_ref[kb, pl.ds(pl.multiple_of(h * DA, DA), DA), kc * KC:(kc + 1) * KC]
        d = _nn(vt, p)
        return (d if acc is None else acc + d), lneg

    def a_finish(h, qb, acc, lneg):
        o = acc * _recip(-jnp.sum(lneg, axis=0, keepdims=True))
        ot_ref[qb, pl.ds(pl.multiple_of(h * DA, DA), DA), :] = o.astype(BF)

    def a_head(h, hpos, state, extra=None):
        acc, lneg, m1, m2 = state
        for qb in range(NQB):
            pos = hpos * NQB + qb
            live = pos < NU
            if live:
                qh = qt_ref[qb, pl.ds(pl.multiple_of(h * DA, DA), DA), :]
            mrun = None
            for c in range(NKC):
                if live:
                    mrun = a_pass1(qh, sbufs[pos % 2], c, mrun)
                    if qb == NQB - 1 and hpos < HA - 1:
                        k_stage(h + 1, c)
                if c < LAG:
                    back, c2, m = 2, NKC - LAG + c, m2
                else:
                    back, c2, m = 1, c - LAG, m1
                if 0 <= pos - back < NU:
                    h2 = h if qb - back >= 0 else h - 1
                    if c2 == 0:
                        acc, lneg = None, None
                    acc, lneg = a_pass2(h2, sbufs[(pos - back) % 2], c2, m, acc, lneg)
                    if c2 == NKC - 1:
                        a_finish(h2, (qb - back) % NQB, acc, lneg)
                if extra is not None:
                    extra(qb * NKC + c)
            m2 = m1
            m1 = jnp.max(mrun, axis=0, keepdims=True) if live else None
            if not live and pos >= NU + 1:
                break
        return acc, lneg, m1, m2

    bscale = (DB ** -0.5) * LOG2E
    ri = lax.broadcasted_iota(jnp.int32, (SEG + MEM, SEG + MEM), 0)
    ci = lax.broadcasted_iota(jnp.int32, (SEG + MEM, SEG + MEM), 1)
    keep = (ri >= SEG) | (ci >= SEG) | (ci <= ri)

    class Step:
        def __init__(self, s, mem):
            self.r0 = pl.multiple_of(s * SEG, SEG)
            self.l0 = pl.multiple_of(s * MEM, MEM)
            xs = x_ref[pl.ds(self.r0, SEG), :]
            tail = jnp.concatenate([xs[16:SEG, :].astype(F32)[0:8, :], mem], axis=0).astype(BF)
            self.h = jnp.concatenate([xs[0:16, :], tail], axis=0)
            self.st1, self.st2, self.st3, self.st4 = {}, {}, {}, {}
            self.acc = None

        def project(self, g):
            out = []
            for hd in range(g * G, (g + 1) * G):
                qkv = _nn(self.h, pltpu.bitcast(w3[hd], BF))
                late = [ql_ref[t, hd, pl.ds(self.l0, MEM), :].astype(F32) for t in range(3)]
                q = qkv[:, 0:128] * bscale
                k = qkv[:, 128:256]
                v = qkv[:, 256:384]
                out.append(tuple(
                    jnp.concatenate([a[0:NE], late[t], a[NE:SEG]], axis=0)
                    for t, a in enumerate((q, k, v))))
            self.st1[g] = out

        def scores(self, g):
            out = []
            for q, k, v in self.st1.pop(g):
                sc = jnp.where(keep, _nt(q, k), -1e9 * LOG2E)
                out.append((sc, jnp.max(sc, axis=1, keepdims=True), v))
            self.st2[g] = out

        def exps(self, g):
            out = []
            for sc, mx, v in self.st2.pop(g):
                e = jnp.exp2(sc - mx)
                out.append((e, jnp.sum(e, axis=1, keepdims=True), v))
            self.st3[g] = out

        def values(self, g):
            out = []
            for e, l, v in self.st3.pop(g):
                o = _nn(e, v)
                out.append((o, _recip(l)))
            self.st4[g] = out

        def output(self, g):
            for k, (o, r) in enumerate(self.st4.pop(g)):
                hd = g * G + k
                on = o * r
                ol_ref[pl.ds(self.l0, MEM), hd * 128:(hd + 1) * 128] = on[NE:SEG].astype(BF)
                oc = jnp.concatenate([on[0:NE], on[SEG:SEG + MEM]], axis=0).astype(BF)
                d = _nn(oc, pltpu.bitcast(wo2[hd], BF))
                self.acc = d if self.acc is None else self.acc + d

        def slot(self, t):
            for lag, stage in enumerate(
                    (self.project, self.scores, self.exps, self.values, self.output)):
                if 0 <= t - lag < NG:
                    stage(t - lag)

        def finish(self):
            b_ref[pl.ds(self.r0, NE), :] = self.acc[0:NE, :]
            return self.acc[NE:SEG, :].astype(BF).astype(F32)

    class TwoSteps:
        def __init__(self, s0, mem):
            self.s0, self.mem, self.k, self.cur = s0, mem, 0, None

        def upto(self, n):
            while self.k < min(n, 2 * NBS):
                step, t = divmod(self.k, NBS)
                if t == 0:
                    self.cur = Step(self.s0 + step, self.mem)
                self.cur.slot(t)
                if t == NBS - 1:
                    self.mem = self.cur.finish()
                self.k += 1

    for c in range(NKC):
        k_stage(0, c)

    def first_extra(slot):
        if slot == 31:
            b_copies[0].wait()
        if slot >= 32:
            relayout_w(slot - 32, 0)

    state = a_head(0, 0, (None, None, None, None), extra=first_extra)

    for s in range(NSEG):
        xl_ref[s * MEM:(s + 1) * MEM, :] = x_ref[s * SEG + NE:(s + 1) * SEG, :]

    for t in range(3):
        b_copies[t + 1].wait()

        def late_qkv(i, carry, t=t):
            for u in range(UL):
                hd0 = (i * UL + u) * 4
                w = jnp.concatenate(
                    [pltpu.bitcast(w3[hd0 + n, :, t * 128:(t + 1) * 128], BF) for n in range(4)],
                    axis=1)
                r = _nn(xl_ref[...], w)
                if t == 0:
                    r = r * bscale
                r = r.astype(BF)
                for n in range(4):
                    ql_ref[t, hd0 + n] = r[:, n * 128:(n + 1) * 128]
                for n in range(4):
                    if t < 2:
                        relayout_w(hd0 + n, t + 1)
                    else:
                        relayout_o(hd0 + n)
            return carry

        lax.fori_loop(0, HB // (4 * UL), late_qkv, 0)

    def head_and_two_steps(h, carry):
        state, mem = carry
        chain = TwoSteps(2 * (h - 1), mem)
        state = a_head(
            h, 1, state, extra=lambda slot: chain.upto((slot + 1) * 2 * NBS // (NQB * NKC)))
        chain.upto(2 * NBS)
        return state, chain.mem

    state, mem = lax.fori_loop(1, HA, head_and_two_steps, (state, mem0_ref[...].astype(F32)))
    chain = TwoSteps(2 * (HA - 1), mem)
    a_head(HA, HA, state, extra=lambda slot: chain.upto(slot + 1))
    chain.upto(2 * NBS)

    bl = None
    for hd in range(HB):
        d = _nn(ol_ref[:, hd * 128:(hd + 1) * 128], pltpu.bitcast(wo2[hd], BF))
        bl = d if bl is None else bl + d
    bl_ref[...] = bl
    for s in range(NSEG):
        b_ref[s * SEG + NE:(s + 1) * SEG, :] = bl_ref[s * MEM:(s + 1) * MEM, :]

    wo_copy.wait()
    for fb in range(NFB):
        qb, c0 = divmod(fb * FB, QB)
        rows = slice(fb * FB, (fb + 1) * FB)
        a = _tn(ot_ref[qb, :, c0:c0 + FB], wo_ref[...])
        gt = jnp.concatenate([gate_ref[rows, :]] * 4, axis=1)
        o_ref[rows, :] = (gt * a + (1.0 - gt) * b_ref[rows, :]).astype(o_ref.dtype)
        o_copy(fb).start()
    for fb in range(NFB):
        o_copy(fb).wait()


def pallas_gated_mix__mha_block__memory_aug_recurrent_mem_tr__prompt_kernel(
        A_x, A_wqkv, A_wo, B_x, B_mem0, B_Wq, B_Wk, B_Wv, B_Wo, B_seg_len, gate_w):
    del B_x
    assert A_x.shape == (1, S_, D_) and B_mem0.shape == (1, MEM, D_) and B_seg_len == SEG
    assert B_Wq.shape == (D_, HB, DB) and B_Wo.shape == (HB, DB, D_)
    x = A_x.reshape(S_, D_)
    mem0 = B_mem0.reshape(MEM, D_)
    wq, wk, wv = (w.reshape(NCH, D_ * HB // NCH, DB) for w in (B_Wq, B_Wk, B_Wv))
    vm = pl.BlockSpec(memory_space=pltpu.VMEM)
    hbm = pl.BlockSpec(memory_space=pl.ANY)
    out = pl.pallas_call(
        _kernel,
        out_shape=jax.ShapeDtypeStruct((S_, D_), A_x.dtype),
        in_specs=[hbm, hbm, hbm, vm, vm, hbm, hbm, hbm, hbm],
        out_specs=hbm,
        scratch_shapes=[
            pltpu.VMEM((S_, D_), BF),
            pltpu.VMEM((D_, 3 * D_), BF),
            pltpu.VMEM((D_, D_), BF),
            pltpu.VMEM((S_, D_), BF),
            pltpu.VMEM((NCH, D_ * HB // NCH, DB), BF),
            pltpu.VMEM((NCH, D_ * HB // NCH, DB), BF),
            pltpu.VMEM((NCH, D_ * HB // NCH, DB), BF),
            pltpu.VMEM((HB, DB, D_), BF),
            pltpu.VMEM((HB, D_ // 2, 3 * DB), U32),
            pltpu.VMEM((HB, DB // 2, D_), U32),
            pltpu.VMEM((NQB, D_, QB), BF),
            pltpu.VMEM((4, S_ // 2, 128), U32),
            pltpu.VMEM((NQB, D_, QB), BF),
            pltpu.VMEM((NQB, D_, QB), BF),
            pltpu.VMEM((S_, QB), F32),
            pltpu.VMEM((S_, QB), F32),
            pltpu.VMEM((S_ // 2, 128), U32),
            pltpu.VMEM((S_, 128), F32),
            pltpu.VMEM((NL, D_), BF),
            pltpu.VMEM((3, HB, NL, DB), BF),
            pltpu.VMEM((NL, HB * DB), BF),
            pltpu.VMEM((NL, D_), F32),
            pltpu.VMEM((S_, D_), F32),
            pltpu.SemaphoreType.DMA((8,)),
            pltpu.SemaphoreType.DMA((NQB,)),
            pltpu.SemaphoreType.DMA((NFB,)),
        ],
        compiler_params=pltpu.CompilerParams(
            vmem_limit_bytes=100 * 1024 * 1024,
            flags={"XLA_TPU_EVENLY_DISTRIBUTE_CRITICAL_NODES": True}),
    )(x, A_wqkv, A_wo, mem0, gate_w, wq, wk, wv, B_Wo)
    return out.reshape(1, S_, D_)
```
